```python
import os as _os
_os.environ.setdefault("JAX_PLATFORMS", "cpu")
import jax
import jax.numpy as jnp

def _softmax(x, axis=-1):
    return jax.nn.softmax(x, axis=axis)
def _gelu(x):
    return jax.nn.gelu(x, approximate=True)
def _silu(x):
    return jax.nn.silu(x)
def _sigmoid(x):
    return jax.nn.sigmoid(x)
def _layernorm(x, axis=-1, eps=1e-5):
    m = jnp.mean(x, axis=axis, keepdims=True)
    v = jnp.var(x, axis=axis, keepdims=True)
    return (x - m) / jnp.sqrt(v + eps)
def _scatter_add(tgt, idx, src, axis=0):
    return tgt.at[idx].add(src)
def _segment_sum(src, seg, n):
    return jax.ops.segment_sum(src, seg, n)
class _Rng:
    def __init__(self, key):
        self._k = key
    def _next(self):
        self._k, sub = jax.random.split(self._k)
        return sub
    def normal(self, shape):
        return jax.random.normal(self._next(), shape, dtype=jnp.bfloat16)
    def randint(self, lo, hi, shape):
        return jax.random.randint(self._next(), shape, lo, hi, dtype=jnp.int32)
    def uniform(self, shape, lo=0.0, hi=1.0):
        return jax.random.uniform(self._next(), shape, jnp.bfloat16, lo, hi)
    def permutation(self, n):
        return jax.random.permutation(self._next(), n)


kernel_name = 'gated_mix__compressed_kv_cla__ssm_conv_h3__prompt'

def setup_inputs():
    _rng = _Rng(jax.random.key(int.from_bytes(__import__("os").urandom(4), "little")))
    _w = (lambda a: (lambda t: t.astype(jnp.bfloat16) if jnp.issubdtype(t.dtype, jnp.floating) else t)(jnp.asarray(a)))
    def _A_setup():
        B, H, Sq, Sk, D, M = 1, 32, 2048, 2048, 128, 1024
        Dc = 4 * D
        return {
            "x": _w((lambda *s: _rng.normal(s) * 0.05)(B, Sq, M)),
            "c_kv": _w((lambda *s: _rng.normal(s) * 0.8)(B, Sk, Dc)),
            "w_q": _w((lambda *s: _rng.normal(s) * 3.2)(M, H, D) * (M ** -0.5)),
            "w_uk": _w((lambda *s: _rng.normal(s) * 3.2)(Dc, H, D) * (Dc ** -0.5)),
            "w_uv": _w((lambda *s: _rng.normal(s) * 0.8)(Dc, H, D) * (Dc ** -0.5)),
            "w_o": _w((lambda *s: _rng.normal(s) * 0.8)(H, D, M) * ((H * D) ** -0.5)),
        }
    _A_in = _A_setup()

    def _B_setup():
        B, S, D = 1, 2048, 1024
        ks = 4
        return {
            "q": _w((lambda *s: _rng.normal(s) * 0.05)(B, S, D)),
            "k": _w((lambda *s: _rng.normal(s) * 0.8)(B, S, D)),
            "v": _w((lambda *s: _rng.normal(s) * 0.8)(B, S, D)),
            "shift_k": _w((lambda *s: _rng.normal(s) * 0.8)(D, ks) * 0.5),
            "ssm_k": _w((lambda *s: _rng.normal(s) * 0.8)(D, S) * (1.0 / S ** 0.5)),
            "ssm_D": _w((lambda *s: _rng.normal(s) * 0.8)(D)),
        }
    _B_in = _B_setup()

    return {
        "A_x": _A_in["x"],
        "A_c_kv": _A_in["c_kv"],
        "A_w_q": _A_in["w_q"],
        "A_w_uk": _A_in["w_uk"],
        "A_w_uv": _A_in["w_uv"],
        "A_w_o": _A_in["w_o"],
        "B_q": _B_in["q"],
        "B_k": _B_in["k"],
        "B_v": _B_in["v"],
        "B_shift_k": _B_in["shift_k"],
        "B_ssm_k": _B_in["ssm_k"],
        "B_ssm_D": _B_in["ssm_D"],
        "gate_w": _w((lambda *s: _rng.normal(s) * 0.05)(1024) * 16.0),
    }

def reference(A_x, A_c_kv, A_w_q, A_w_uk, A_w_uv, A_w_o, B_q, B_k, B_v, B_shift_k, B_ssm_k, B_ssm_D, gate_w):
    def _A_ref(x, c_kv, w_q, w_uk, w_uv, w_o):
        B, Sq, M = x.shape[0], x.shape[1], x.shape[2]
        Sk = c_kv.shape[1]
        H, D = w_q.shape[1], w_q.shape[2]
        q = jnp.einsum("bqm,mhd->bhqd", x, w_q)
        k = jnp.einsum("bkc,chd->bhkd", c_kv, w_uk)
        v = jnp.einsum("bkc,chd->bhkd", c_kv, w_uv)
        scores = jnp.einsum("bhqd,bhkd->bhqk", q, k) * (D ** -0.5)
        off = Sk - Sq
        qi = jnp.arange(Sq)[:, None]
        kj = jnp.arange(Sk)[None, :]
        cmask = kj <= (qi + off)
        scores = jnp.where(cmask[None, None], scores, -1e9)
        p = _softmax(scores, axis=-1)
        ctx = jnp.einsum("bhqk,bhkd->bhqd", p, v)
        return jnp.einsum("bhqd,hdm->bqm", ctx, w_o)

    def _B_ref(q, k, v, shift_k, ssm_k, ssm_D):
        B, S, D = q.shape
        ks = shift_k.shape[-1]
        k_pad = jnp.pad(k, ((0, 0), (ks - 1, 0), (0, 0)))
        k_shift = jnp.zeros_like(k)
        for t in range(ks):
            k_shift = k_shift + k_pad[:, t:t + S, :] * shift_k[:, ks - 1 - t][None, None, :]
        kv = k_shift * v
        L = 2 * S
        kv_pad = jnp.pad(kv, ((0, 0), (0, S), (0, 0)))
        kf_pad = jnp.pad(ssm_k, ((0, 0), (0, S)))
        kv_f = (lambda x, axes=(-2,-1): jnp.fft.rfft2(x.astype(jnp.float32), axes=axes))(kv_pad[:, None, :, :], axes=(1, 2))
        kf_f = (lambda x, axes=(-2,-1): jnp.fft.rfft2(x.astype(jnp.float32), axes=axes))(kf_pad[:, None, :], axes=(1, 2))
        kf_f = (lambda x, *d: x.transpose(*d))(kf_f, 1, 2, 0)
        y_f = kv_f * kf_f[None, :, :, :]
        y = (lambda x, s, axes=(-2,-1): jnp.fft.irfft2(x, s=s, axes=axes).astype(jnp.bfloat16))(y_f, (1, L), axes=(1, 2))[:, 0, :S, :]
        y = y + kv * ssm_D[None, None, :]
        return q * y

    x = A_x
    g = _sigmoid((x * gate_w).sum(-1, keepdims=True))
    a = _A_ref(x, A_c_kv, A_w_q, A_w_uk, A_w_uv, A_w_o)
    b = _B_ref(x, B_k, B_v, B_shift_k, B_ssm_k, B_ssm_D)
    return g * a + (1 - g) * b
```

```python
import math

import jax
import jax.numpy as jnp
from jax import lax
from jax.experimental import pallas as pl
from jax.experimental.pallas import tpu as pltpu

OPT = {}

S = 2048
M = 1024
H = 32
D = 128
DC = 512
KS = 4
T = 128
C = 128
P = S // C
NCB = M // T
HG = 8
NG = H // HG
BQ = int(OPT.get('bq', 256))
BP = int(OPT.get('bp', 128))
BO = int(OPT.get('bo', 128))
RC = int(OPT.get('rc', 32))
NC = T // RC
DELAY = int(OPT.get('delay', 2))
ELAG = int(OPT.get('elag', 0))
XLAG = int(OPT.get('xlag', 3))
LAG = int(OPT.get('lag', 5))
MLAG = int(OPT.get('mlag', 1))
NX = int(OPT.get('nx', 2))
SEM_C, SEM_KV, SEM_Q, SEM_S, SEM_B, SEM_O, SEM_X = range(7)
MB = int(OPT.get('mb', 2))

A_CTX = 0
A_X = A_CTX + H
A_CKV = A_X + NCB
A_OUT = A_CKV + DC // T
A_SPEC = A_OUT + NCB
A_GATE = A_SPEC + 4
A_TOK = A_GATE + 2
A_P = A_TOK + 1
A_S = A_P + 1
A_U = A_S
A_G = A_S + 4
A_STG = A_S + 8
A_W = A_STG + 1
A_END = A_W + H
RING = 64
B_Q, B_K, B_V = 0, 1, 2

F32 = jnp.float32
BF16 = jnp.bfloat16
U32 = jnp.uint32

_NT = (((1,), (1,)), ((), ()))


def _dot(a, b):
    return jnp.dot(a, b, preferred_element_type=F32)


def _dot_nt(a, b):
    return lax.dot_general(a, b, _NT, preferred_element_type=F32)


def _ld(ref, i, r0, n):
    return pltpu.bitcast(ref[i, r0 // 2:(r0 + n) // 2, :], BF16)


def _st(ref, i, r0, val):
    ref[i, r0 // 2:(r0 + val.shape[0]) // 2, :] = pltpu.bitcast(val, U32)


def _tree(op, vals):
    while len(vals) > 1:
        vals = [op(a, b) for a, b in zip(vals[::2], vals[1::2])] + vals[len(vals) // 2 * 2:]
    return vals[0]


class _Pacer:
    def __init__(self, lag=0):
        self.jobs = []
        self.live = []
        self.lag = lag
        self.now = 0
        self.credit = 0.0
        self.rate = 0.0

    def add(self, cost, fn):
        self.jobs.append((cost, fn))

    def spread(self, ticks):
        self.rate = sum(c for c, _ in self.jobs) / ticks
        self.credit = 0.0

    def tick(self):
        self.now += 1
        while self.live and self.live[0][0] <= self.now:
            self.live.pop(0)[1]()
        self.credit += self.rate
        while self.jobs and self.jobs[0][0] <= self.credit + 1e-6:
            cost, fn = self.jobs.pop(0)
            self.credit -= cost
            fin = fn()
            if fin is not None:
                self.live.append((self.now + self.lag, fin))

    def flush(self):
        while self.jobs:
            fin = self.jobs.pop(0)[1]()
            if fin is not None:
                self.live.append((0, fin))
        while self.live:
            self.live.pop(0)[1]()


class _Stream:
    def __init__(self, pacers=()):
        self.pos = 0
        self.events = {}
        self.pacers = pacers

    def at(self, slot, fn, first=False):
        assert slot >= NC * self.pos, (slot, self.pos)
        lst = self.events.setdefault(slot, [])
        lst.insert(0 if first else len(lst), fn)

    def step(self, load, mm, sink):
        chunks = []
        for c in range(NC):
            for fn in self.events.pop(NC * self.pos + c, ()):
                fn()
            if self.pos >= DELAY:
                for p in self.pacers:
                    p.tick()
            chunks.append(load(c * RC))
        res = mm([jnp.concatenate(col, axis=0) for col in zip(*chunks)])
        for c in range(NC):
            self.at(NC * (self.pos + DELAY) + c,
                    lambda r=c * RC: sink(r, [v[r:r + RC] for v in res]), first=True)
        self.pos += 1

    def drain(self):
        for slot in sorted(self.events):
            for fn in self.events.pop(slot):
                fn()
        for p in self.pacers:
            p.flush()


RR = 32


def _repack_job(raw, act, g, r, row0, k):
    base = (k % 8) * RR * HG // 2

    def stage():
        blk = raw[g, pl.ds(pl.multiple_of(r, RR), RR)]
        act[A_STG, base:base + RR * HG // 2, :] = pltpu.bitcast(blk.reshape(RR * HG, D), U32)

    def split():
        out = pl.ds(pl.multiple_of((row0 + r) // 2, RR // 2), RR // 2)
        vals = []
        for hp in range(HG // 2):
            ev = act[A_STG, pl.ds(base + hp, RR // 2, stride=HG), :]
            od = act[A_STG, pl.ds(base + HG // 2 + hp, RR // 2, stride=HG), :]
            vals += [(ev & U32(0xFFFF)) | (od << 16), (ev >> 16) | (od & U32(0xFFFF0000))]

        def fin():
            for i, v in enumerate(vals):
                act[A_W + g * HG + i, out, :] = v
        return fin

    return [stage, split]


def _head_stream(opd, act, tok, h, fillers):
    tri = (lax.broadcasted_iota(jnp.int32, (T, T), 1) <= lax.broadcasted_iota(jnp.int32, (T, T), 0))
    strips = list(range(S // T))
    if OPT.get('order', 'desc') == 'desc':
        strips = strips[::-1]
    elif OPT.get('order') == 'mix':
        strips = [j for a in range(S // T // 2) for j in (a, S // T - 1 - a)]
    elif OPT.get('order') == 'mix2':
        strips = [j for a in range(S // T // 2) for j in (S // T - 1 - a, a)]
    tiles = [(j, t) for j in strips for t in range(j + 1)]
    index = {jt: i for i, jt in enumerate(tiles)}
    groups = []
    for g in range(len(tiles) // 4):
        segs = []
        for j, t in tiles[4 * g:4 * g + 4]:
            if segs and segs[-1][0] == j:
                segs[-1][2] += 1
            else:
                segs.append([j, t, t + 1])
        groups.append(segs)
    ng = len(groups)

    def s_at(j, t, r):
        i = index[(j, t)] % RING
        return A_S + i // 8, slice((i % 8) * T + r, (i % 8) * T + r + RC), slice(None)

    def p_at(j, t, r):
        i = index[(j, t)] % 16
        return A_P, slice((i * T + r) // 2, (i * T + r + RC) // 2), slice(None)

    RELOAD = OPT.get('reload', '1') == '1'
    kept = {}

    def pin(k, r, val):
        act[tok, k * T + r:k * T + r + RC, :] = pltpu.bitcast(val, U32)
        kept[(k, r)] = val

    def pinned(k, r):
        return pltpu.bitcast(act[tok, k * T + r:k * T + r + RC, :], F32) if RELOAD else kept[(k, r)]

    row_max, inv_sum, probs = {}, {}, {}

    def qk_step(st, g):
        def sink(r, res):
            for (j, t0, t1), s in zip(groups[g], res):
                vs = []
                for t in range(t0, t1):
                    v = s[:, (t - t0) * T:(t - t0 + 1) * T]
                    if t == j:
                        v = jnp.where(tri[r:r + RC], v, -1e30)
                    act[s_at(j, t, r)] = pltpu.bitcast(v, U32)
                    vs.append(v)
                m = _tree(jnp.maximum, vs)
                if t0 > 0:
                    m = jnp.maximum(m, pinned(0, r))
                if t1 == j + 1:
                    row_max[(j, r)] = jnp.max(m, axis=1, keepdims=True)
            pin(0, r, m)

        st.step(lambda r: [_ld(opd, B_Q, j * T + r, RC) for j, _, _ in groups[g]],
                lambda qs: [_dot_nt(q, _ld(opd, B_K, t0 * T, (t1 - t0) * T))
                            for q, (_, t0, t1) in zip(qs, groups[g])], sink)

    def exp_job(st, g, r, slot):
        def start():
            out = []
            for j, t0, t1 in groups[g]:
                ps = [jnp.exp2(pltpu.bitcast(act[s_at(j, t, r)], F32) - row_max[(j, r)]) for t in range(t0, t1)]
                out.append(jnp.concatenate(ps, axis=1))
                l = _tree(jnp.add, ps)
                if t0 > 0:
                    l = l + pinned(1, r)
                if t1 == j + 1:
                    inv_sum[(j, r)] = pltpu.reciprocal(jnp.sum(l, axis=1, keepdims=True), full_range=False)
            probs[(g, r)] = out
            st.at(slot + ELAG + 1, lambda: pin(1, r, l))

        st.at(slot, start)

    def pv_step(st, g):
        def sink(r, res):
            for (j, t0, t1), o in zip(groups[g], res):
                if t0 > 0:
                    o = o + pinned(2, r)
                if t1 == j + 1:
                    _st(act, A_CTX + h, j * T + r, (o * inv_sum.pop((j, r))).astype(BF16))
                else:
                    pin(2, r, o)

        st.step(lambda r: probs.pop((g, r)),
                lambda ps: [_dot(p.astype(BF16), _ld(opd, B_V, t0 * T, (t1 - t0) * T))
                            for p, (_, t0, t1) in zip(ps, groups[g])], sink)

    need = [index[(groups[g][-1][0], groups[g][-1][0])] // 4 for g in range(ng)]
    lead = ELAG
    seq, posq = [], {}
    gq = gp = 0
    fillers = list(fillers)
    while gp < ng:
        ok = need[gp] in posq and NC * (posq[need[gp]] + DELAY) + XLAG <= NC * len(seq) - lead
        other = gq < ng or bool(fillers)
        if (ok and (not other or seq[-1][0] != 'p')) or not other:
            seq.append(('p', gp))
            gp += 1
        elif gq < ng:
            posq[gq] = len(seq)
            seq.append(('q', gq))
            gq += 1
        else:
            seq.append(('f', fillers.pop(0)))
        assert (gq - gp) * 4 <= RING
    seq += [('f', f) for f in fillers]

    st = _Stream()
    for pos, (kind, g) in enumerate(seq):
        if kind == 'p':
            for c in range(NC):
                exp_job(st, g, c * RC, max(NC * pos + c - lead, NC * (posq[need[g]] + DELAY) + c))
    for kind, g in seq:
        if kind == 'q':
            qk_step(st, g)
        elif kind == 'p':
            pv_step(st, g)
        else:
            g(st)
    st.drain()


def _kernel(x_hbm, ckv_hbm, wq_hbm, wuk_hbm, wuv_hbm, wo_hbm, bk_hbm, bv_hbm, sk_hbm,
            shift_hbm, ssmd_hbm, gate_hbm, out_hbm,
            act_v, opd, wq_v, wuk_v, wuv_v, wo_v, bk_v, bv_v, sk_v, shift_ref, ssmd_ref, gate_ref,
            f_v, fi_v, kpad_v, par_v, zero_s, sems):
    def lanes(i):
        return pl.ds(i * T, T)

    def start(copies):
        for c in copies:
            c.start()

    def wait(copies):
        for c in copies:
            c.wait()

    def x_cp(k):
        rows = pl.ds(k * (S // NX), S // NX)
        return [pltpu.make_async_copy(x_hbm.at[rows, lanes(i)], act_v.at[A_X + i, rows], sems.at[SEM_X + k])
                for i in range(NCB)]

    def c_cp():
        return [pltpu.make_async_copy(ckv_hbm.at[:, lanes(i)], act_v.at[A_CKV + i], sems.at[SEM_C])
                for i in range(DC // T)]

    def wkv_cp(g):
        return [pltpu.make_async_copy(src.at[:, pl.ds(g * HG, HG), :], dst.at[g], sems.at[SEM_KV])
                for src, dst in ((wuk_hbm, wuk_v), (wuv_hbm, wuv_v))]

    def wq_cp(g):
        return [pltpu.make_async_copy(wq_hbm.at[:, pl.ds(g * HG, HG), :], wq_v.at[g], sems.at[SEM_Q])]

    def small_cp():
        return [pltpu.make_async_copy(src, dst, sems.at[SEM_S])
                for src, dst in ((shift_hbm, shift_ref), (ssmd_hbm, ssmd_ref), (gate_hbm, gate_ref))]

    def b_cp():
        return [pltpu.make_async_copy(src, dst, sems.at[SEM_B]) for i in range(NCB) for src, dst in (
            (bk_hbm.at[:, lanes(i)], bk_v.at[i]), (bv_hbm.at[:, lanes(i)], bv_v.at[i]),
            (sk_hbm.at[lanes(i), :], sk_v.at[i]), (wo_hbm.at[:, lanes(i)], wo_v.at[i]))]

    start(small_cp() + wkv_cp(0) + c_cp())

    def phase(fidx, n):
        return (((2 * fidx + 1) * n) & (4 * C - 1)).astype(F32) * (math.pi / (2 * C))

    r = lax.broadcasted_iota(jnp.int32, (C, C), 0)
    c_ = lax.broadcasted_iota(jnp.int32, (C, C), 1)
    th = phase(r, c_)
    f_v[0:C, :] = jnp.cos(th).astype(BF16)
    f_v[C:2 * C, :] = (-jnp.sin(th)).astype(BF16)
    th = phase(c_, r)
    fi_v[:, 0:C] = (jnp.cos(th) * (1.0 / C)).astype(BF16)
    fi_v[:, C:2 * C] = (-jnp.sin(th) * (1.0 / C)).astype(BF16)
    kpad_v[0:8, :] = jnp.zeros((8, T), F32)
    wait(small_cp())
    start(wq_cp(0))
    sh = shift_ref[...].astype(F32)
    dd = ssmd_ref[...].astype(F32)
    for cb in range(NCB):
        par_v[cb, 0:KS, :] = sh[:, cb * T:(cb + 1) * T]
        par_v[cb, KS:KS + 1, :] = dd[cb:cb + 1, :]
    zero_s[0] = 0

    act = act_v.bitcast(U32)
    wo_u = wo_v.bitcast(U32)
    qscale = (D ** -0.5) * math.log2(math.e)

    NSL = 4

    def repack(g, j, which=(0, 1, 2)):
        jobs = []
        for w in which:
            raw, rows, row0 = ((wq_v, M, 0), (wuk_v, DC, M), (wuv_v, DC, M + DC))[w]
            for r in range(0, rows // NSL, RR):
                jobs += _repack_job(raw, act, g, j * (rows // NSL) + r, row0, len(jobs) // 2)
        return jobs

    def q_steps(h, tok, pacer, first, n0=0, n1=2 * S // T):
        w = {}
        half = {}

        def step(st, n):
            k, r0 = n % 2, n // 2 * T
            if n == n0:
                w.update({i: _ld(act, A_W + h, i * DC, DC) for i in range(2)})
            if n == first:
                pacer.spread((n1 - 2 - first) * NC - pacer.lag)
                st.pacers = [pacer]
            if n == n1 - 1:
                assert not pacer.jobs and not pacer.live

            def sink(r, res):
                if n < n1 - 1 - DELAY:
                    act[tok, 3 * T:3 * T + 8, :] = pltpu.bitcast(res[0][0:8], U32)
                if k == 0:
                    half[r0 + r] = res[0]
                else:
                    _st(opd, B_Q, r0 + r, ((half.pop(r0 + r) + res[0]) * qscale).astype(BF16))

            st.step(lambda r: [jnp.concatenate([_ld(act, A_X + 4 * k + i, r0 + r, RC) for i in range(4)], axis=1)],
                    lambda lhs: [_dot(lhs[0], w[k])], sink)

        return [lambda st, n=n: step(st, n) for n in range(n0, n1)]

    def kv_project(h, between=None):
        for dst, row in ((B_K, M), (B_V, M + DC)):
            if dst == B_V and between:
                between()
            c = jnp.concatenate([_ld(act, A_CKV + i, 0, S) for i in range(4)], axis=1)
            _st(opd, dst, 0, _dot(c, _ld(act, A_W + h, row, DC)).astype(BF16))

    def repack_first(which):
        def body(j, carry):
            jobs = repack(0, j, which)
            for job in jobs[::2]:
                job()
            for job in jobs[1::2]:
                job()()
            return carry

        lax.fori_loop(0, NSL, body, 0)

    with jax.named_scope("wait1"):
        wait(wkv_cp(0))
    start(x_cp(0))
    with jax.named_scope("rp1"):
        repack_first((1, 2))
    with jax.named_scope("wait2"):
        wait(c_cp())
    with jax.named_scope("kv0"):
        kv_project(0, lambda: [start(x_cp(k)) for k in range(1, NX)])
    with jax.named_scope("wait3"):
        wait(wq_cp(0))
    repack_first((0,))
    gw = gate_ref[...].astype(F32)

    def gate_job(r0):
        acc = None
        for i in range(NCB):
            t = _ld(act, A_X + i, r0, 16).astype(F32) * gw[i:i + 1, :]
            acc = t if acc is None else acc + t
        g = jax.nn.sigmoid(jnp.sum(acc, axis=1, keepdims=True))

        def fin():
            act[A_GATE + r0 // (S // 2), r0 % (S // 2):r0 % (S // 2) + 16, :] = pltpu.bitcast(
                jnp.broadcast_to(g, (16, T)), U32)
        return fin

    for k in range(NX):
        with jax.named_scope("wait4"):
            wait(x_cp(k))
        if k == NX - 1:
            start(wkv_cp(1) + wq_cp(1))
        with jax.named_scope("q0"):
            pacer = _Pacer(LAG)
            for r0 in range(k * S // NX, (k + 1) * S // NX, 16):
                pacer.add(1, lambda r0=r0: gate_job(r0))
            st = _Stream()
            n0 = k * (2 * S // T // NX)
            for f in q_steps(0, zero_s[0] + A_TOK, pacer, n0 + DELAY, n0, n0 + 2 * S // T // NX):
                f(st)
            st.drain()

    def head(h, carry):
        side = _Pacer(1)
        for job in repack(jnp.minimum((h + NSL - 1) // NSL, NG - 1), (h + NSL - 1) % NSL):
            side.add(1, job)
        tok = zero_s[0] + A_TOK
        _head_stream(opd, act, tok, h, q_steps(h + 1, tok, side, 9))
        kv_project(h + 1)
        return carry

    def head_group(gi, carry):
        for g in range(1, NG):
            @pl.when(gi == g)
            def _():
                wait(wkv_cp(g) + wq_cp(g))
                start(wkv_cp(g + 1) + wq_cp(g + 1) if g + 1 < NG else b_cp())

        return lax.fori_loop(jnp.maximum((gi - 1) * NSL + 1, 0), jnp.where(gi == NG - 1, H - 1, gi * NSL + 1),
                             head, carry)

    if not OPT.get('nohead'):
      with jax.named_scope("heads"):
        lax.fori_loop(0, NG, head_group, 0)
      with jax.named_scope("last"):
        _head_stream(opd, act, zero_s[0] + A_TOK, zero_s[0] + H - 1, [])
    wait(b_cp())

    def o_cp(i):
        return pltpu.make_async_copy(act_v.at[A_OUT + i], out_hbm.at[:, pl.ds(pl.multiple_of(i * T, T), T)],
                                     sems.at[SEM_O])

    def spec_at(base, a, r, n):
        return base + a // 4, slice((a % 4) * 2 * C + r, (a % 4) * 2 * C + r + n), slice(None)

    def out_block(cb, carry):
        kpad_v[8:8 + S, :] = bk_v[cb].astype(F32)
        sgn = (1 - 2 * (lax.broadcasted_iota(jnp.int32, (C, T), 0) & 1)).astype(F32)
        prev = None
        for d0 in range(0, P, 4):
            hk = jnp.concatenate([sk_v[cb, :, d * C:(d + 1) * C] for d in range(d0, d0 + 4)], axis=0)
            hf = _dot_nt(f_v[...], hk)
            for k in range(4):
                cur = hf[0:C, k * T:(k + 1) * T], hf[C:2 * C, k * T:(k + 1) * T]
                if prev is None:
                    re, im = cur[0] + par_v[cb, KS:KS + 1, :], cur[1]
                else:
                    re, im = cur[0] - sgn * prev[1], cur[1] + sgn * prev[0]
                prev = cur
                act[spec_at(A_G, d0 + k, 0, C)] = pltpu.bitcast(re, U32)
                act[spec_at(A_G, d0 + k, C, C)] = pltpu.bitcast(im, U32)
            kvs = []
            for a in range(d0, d0 + 4):
                acc = None
                for j in range(KS):
                    t = kpad_v[pl.ds(8 + a * C - j, C), :] * par_v[cb, j:j + 1, :]
                    acc = t if acc is None else acc + t
                kvs.append((acc * bv_v[cb, a * C:(a + 1) * C, :].astype(F32)).astype(BF16))
            uf = _dot(f_v[...], jnp.concatenate(kvs, axis=1))
            for k in range(4):
                act[spec_at(A_U, d0 + k, 0, 2 * C)] = pltpu.bitcast(uf[:, k * T:(k + 1) * T], U32)

        done = []
        part = {}

        def spec(base, a, f0):
            return [pltpu.bitcast(act[spec_at(base, a, o + f0, 8)], F32) for o in (0, C)]

        def mac(a, f0, b0, b1):
            acc = part.pop((a, f0), {})
            gs = {d: spec(A_G, d, f0) for d in range(max(a - b1, 0), a - b0 + 1)}
            for b in range(b0, b1):
                ur, ui = spec(A_U, b, f0)
                for o in (a, a - 1):
                    if b <= o:
                        gr, gi = gs[o - b]
                        t = ur * gr - ui * gi, ur * gi + ui * gr
                        acc[o] = (acc[o][0] + t[0], acc[o][1] + t[1]) if o in acc else t
            if b1 <= a:
                part[(a, f0)] = acc
            vals = dict(acc)

            def fin():
                for o, (yr, yi) in vals.items():
                    act[spec_at(A_SPEC, o, f0, 8)] = pltpu.bitcast(yr, U32)
                    act[spec_at(A_SPEC, o, C + f0, 8)] = pltpu.bitcast(yi, U32)
                if f0 == C - 8 and b1 > a:
                    done.extend((a, a - 1))
            return fin

        pacer, mixer = _Pacer(MLAG), _Pacer(MLAG)
        for a in range(P - 1, 0, -2):
            for f0 in range(0, C, 8):
                for b0 in range(0, a + 1, MB):
                    b1 = min(b0 + MB, a + 1)
                    pacer.add(b1 - b0, lambda arg=(a, f0, b0, b1): mac(*arg))
        pacer.spread((P - 2) * (H // 4) * NC - DELAY * NC - MLAG - 2)
        mixer.rate = 0.5
        st = _Stream([pacer, mixer])
        tok = zero_s[0] + A_TOK
        attn, conv, run = {}, {}, {}

        def mix(r0, av, yv):
            x = _ld(act, A_X + cb, r0, RC).astype(F32)
            g = pltpu.bitcast(act[A_GATE + r0 // (S // 2), r0 % (S // 2):r0 % (S // 2) + RC, :], F32)
            return lambda: _st(act, A_OUT + cb, r0, (g * av + (1.0 - g) * (x * yv)).astype(BF16))

        def queue_mix(r0):
            if r0 in attn and r0 in conv:
                if not mixer.jobs:
                    mixer.credit = 0.5
                mixer.add(1.0 / max(1, min(3, len(mixer.jobs) // 4)),
                          lambda arg=(r0, attn.pop(r0), conv.pop(r0)): mix(*arg))

        def out_step(a, k):
            def sink(r, res):
                acc = res[0]
                if k > 0:
                    acc = acc + pltpu.bitcast(act[tok, T + r:T + r + RC, :], F32)
                act[tok, T + r:T + r + RC, :] = pltpu.bitcast(acc, U32)
                if k == H // 4 - 1:
                    attn[a * C + r] = acc
                    queue_mix(a * C + r)

            st.step(lambda r: [jnp.concatenate([_ld(act, A_CTX + 4 * k + i, a * C + r, RC) for i in range(4)], axis=1)],
                    lambda lhs: [_dot(lhs[0], _ld(wo_u, cb, k * 4 * D, 4 * D))], sink)

        def inv_step(pair, ys):
            def sink(r, res):
                act[tok, 0:8, :] = pltpu.bitcast(res[0][0:8, 0:T], U32)
                for i, a in enumerate(pair):
                    conv[a * C + r] = res[0][:, i * T:(i + 1) * T]
                    queue_mix(a * C + r)

            st.step(lambda r: [fi_v[r:r + RC, :]], lambda lhs: [_dot(lhs[0], ys)], sink)

        for a in reversed(range(P)):
            for k in range(H // 4):
                pair = None
                if len(done) >= 2:
                    pair = done[:2]
                    del done[:2]
                    ys = jnp.concatenate(
                        [pltpu.bitcast(act[spec_at(A_SPEC, b, 0, 2 * C)], F32).astype(BF16) for b in pair], axis=1)
                out_step(a, k)
                if pair:
                    inv_step(pair, ys)
        assert not pacer.jobs and not pacer.live and not done
        st.drain()
        assert not attn and not conv
        o_cp(cb).start()
        return carry

    if OPT.get('noout'):
        return
    with jax.named_scope("out"):
        lax.fori_loop(0, NCB, out_block, 0)
    for i in range(NCB):
        o_cp(i).wait()


@jax.jit
def pallas_gated_mix__compressed_kv_cla__ssm_conv_h3__prompt_kernel(
    A_x, A_c_kv, A_w_q, A_w_uk, A_w_uv, A_w_o, B_q, B_k, B_v, B_shift_k, B_ssm_k, B_ssm_D, gate_w,
):
    del B_q
    hbm = pl.BlockSpec(memory_space=pl.ANY)
    scratch = [
        pltpu.VMEM((A_END, S, T), BF16), pltpu.VMEM((3, S // 2, D), U32),
        pltpu.VMEM((NG, M, HG, D), BF16), pltpu.VMEM((NG, DC, HG, D), BF16), pltpu.VMEM((NG, DC, HG, D), BF16),
        pltpu.VMEM((NCB, H * D, T), BF16),
        pltpu.VMEM((NCB, S, T), BF16), pltpu.VMEM((NCB, S, T), BF16), pltpu.VMEM((NCB, T, S), BF16),
        pltpu.VMEM((KS, M), BF16), pltpu.VMEM((NCB, T), BF16), pltpu.VMEM((NCB, T), BF16),
        pltpu.VMEM((2 * C, C), BF16), pltpu.VMEM((C, 2 * C), BF16), pltpu.VMEM((S + 8, T), F32),
        pltpu.VMEM((NCB, 8, T), F32),
        pltpu.SMEM((1,), jnp.int32),
        pltpu.SemaphoreType.DMA((SEM_X + NX,)),
    ]
    out = pl.pallas_call(
        _kernel,
        out_shape=jax.ShapeDtypeStruct((S, M), BF16),
        in_specs=[hbm] * 12,
        out_specs=hbm,
        scratch_shapes=scratch,
        compiler_params=pltpu.CompilerParams(
            vmem_limit_bytes=120 * 1024 * 1024,
            flags={k: True for k in OPT.get('flags', '').split('+') if k}),
    )(A_x.reshape(S, M), A_c_kv.reshape(S, DC), A_w_q, A_w_uk, A_w_uv, A_w_o.reshape(H * D, M),
      B_k.reshape(S, M), B_v.reshape(S, M), B_ssm_k,
      B_shift_k.T, B_ssm_D.reshape(NCB, T), gate_w.reshape(NCB, T))
    return out.reshape(1, S, M)
```

```python
import math

import jax
import jax.numpy as jnp
import numpy as np
from jax import lax
from jax.experimental import pallas as pl
from jax.experimental.pallas import tpu as pltpu

S = 2048
M = 1024
H = 32
D = 128
DC = 512
KS = 4
T = 128
C = 128
P = S // C
NCB = M // T
HG = 8
NG = H // HG

RC = 32
NC = T // RC
DELAY = 2
XLAG = 3
HP = 4
HA = 2
RR = 32
MB = 2
MF = 8
RING = 64

PAGE = S // 2
A_Q = 0
A_X = A_Q + H
A_C = A_X + NCB
A_GATE = A_C + DC // T
A_RUN = A_GATE + 2
A_STG = A_RUN + 1
A_W = A_STG + 2
A_S = A_W
A_U, A_G, A_Y = A_W, A_W + 8, A_W + 16
A_END = A_W + H
SEM_C, SEM_KV, SEM_A, SEM_B, SEM_O, SEM_END = range(6)

F32 = jnp.float32
BF16 = jnp.bfloat16
U32 = jnp.uint32


def _dot(a, b):
    return jnp.dot(a, b, preferred_element_type=F32)


def _dot_nt(a, b):
    return lax.dot_general(a, b, (((1,), (1,)), ((), ())), preferred_element_type=F32)


def _ld16(ref, page, r0, n):
    return pltpu.bitcast(ref[page, r0 // 2:(r0 + n) // 2, :], BF16)


def _st16(ref, page, r0, val):
    ref[page, r0 // 2:(r0 + val.shape[0]) // 2, :] = pltpu.bitcast(val.astype(BF16), F32)


def _ld32(ref, page, r0, n):
    return ref[page + r0 // PAGE if r0 >= PAGE else page, r0 % PAGE:r0 % PAGE + n, :]


def _st32(ref, page, r0, val):
    ref[page + r0 // PAGE if r0 >= PAGE else page, r0 % PAGE:r0 % PAGE + val.shape[0], :] = val


def _tree(op, vals):
    while len(vals) > 1:
        vals = [op(a, b) for a, b in zip(vals[::2], vals[1::2])] + vals[len(vals) // 2 * 2:]
    return vals[0]


class _Jobs:
    def __init__(self, lag):
        self.jobs, self.live = [], []
        self.lag, self.now, self.credit, self.rate = lag, 0, 0.0, 0.0

    def add(self, cost, fn):
        self.jobs.append((cost, fn))

    def spread(self, slots):
        self.rate = sum(c for c, _ in self.jobs) / slots

    def idle(self):
        return not self.jobs and not self.live

    def tick(self):
        self.now += 1
        while self.live and self.live[0][0] <= self.now:
            self.live.pop(0)[1]()
        self.credit += self.rate
        while self.jobs and self.jobs[0][0] <= self.credit + 1e-6:
            cost, fn = self.jobs.pop(0)
            self.credit -= cost
            fin = fn()
            if fin is not None:
                self.live.append((self.now + self.lag, fin))

    def flush(self):
        while self.jobs:
            fin = self.jobs.pop(0)[1]()
            if fin is not None:
                self.live.append((0, fin))
        while self.live:
            self.live.pop(0)[1]()


class _Stream:
    def __init__(self, queues=()):
        self.pos = 0
        self.events = {}
        self.queues = queues

    def at(self, slot, fn, first=False):
        assert slot >= NC * self.pos
        lst = self.events.setdefault(slot, [])
        lst.insert(0 if first else len(lst), fn)

    def step(self, load, mm, sink, early=0, first=True):
        chunks = []
        for c in range(NC):
            for fn in self.events.pop(NC * self.pos + c, ()):
                fn()
            if self.pos >= DELAY:
                for q in self.queues:
                    q.tick()
            chunks.append(load(c * RC))
        res = mm([jnp.concatenate(col, axis=0) for col in zip(*chunks)])
        for c in range(NC):
            self.at(NC * (self.pos + DELAY) + c - early, lambda r=c * RC: sink(r, [v[r:r + RC] for v in res]), first)
        self.pos += 1

    def drain(self):
        for slot in sorted(self.events):
            for fn in self.events.pop(slot):
                fn()
        for q in self.queues:
            q.flush()


def _repack_jobs(raw, act, g, r, row0, k):
    page, base = A_STG + k % 8 // 4, k % 4 * (RR * HG // 2)

    def stage():
        blk = raw[g, pl.ds(pl.multiple_of(r, RR), RR)]
        act[page, base:base + RR * HG // 2, :] = pltpu.bitcast(blk.reshape(RR * HG, D), F32)

    def split():
        out = pl.ds(pl.multiple_of((row0 + r) // 2, RR // 2), RR // 2)
        vals = []
        for hp in range(HG // 2):
            ev, od = (pltpu.bitcast(act[page, pl.ds(base + o + hp, RR // 2, stride=HG), :], U32)
                      for o in (0, HG // 2))
            vals += [(ev & np.uint32(0xFFFF)) | (od << 16), (ev >> 16) | (od & np.uint32(0xFFFF0000))]

        def fin():
            for i, v in enumerate(vals):
                act[A_W + g * HG + i, out, :] = pltpu.bitcast(v, F32)
        return fin

    return [stage, split]


def _attention(kv, act, run, heads):
    tri = lax.broadcasted_iota(jnp.int32, (T, T), 1) <= lax.broadcasted_iota(jnp.int32, (T, T), 0)
    nt = S // T
    order = [nt // 2 - 1] + [j for a in reversed(range(nt // 2 - 1)) for j in (a, nt - 2 - a)] + [nt - 1]
    tiles = [((n, j), t) for n in range(len(heads)) for j in order for t in range(j + 1)]
    index = {jt: i for i, jt in enumerate(tiles)}
    groups = []
    for g in range(len(tiles) // 4):
        runs = []
        for j, t in tiles[4 * g:4 * g + 4]:
            if runs and runs[-1][0] == j:
                runs[-1][2] += 1
            else:
                runs.append([j, t, t + 1])
        groups.append(runs)
    ng = len(groups)
    v_page = [H + h for h in heads]
    row_max, inv_sum, probs = {}, {}, {}

    def s_row(j, t, r):
        return index[(j, t)] % RING * T + r

    def qk_step(st, g):
        def sink(r, res):
            for (j, t0, t1), s in zip(groups[g], res):
                vs = []
                for t in range(t0, t1):
                    v = s[:, (t - t0) * T:(t - t0 + 1) * T]
                    if t == j[1]:
                        v = jnp.where(tri[r:r + RC], v, -jnp.inf)
                    _st32(act, A_S, s_row(j, t, r), v)
                    vs.append(v)
                m = _tree(jnp.maximum, vs)
                if t0 > 0:
                    m = jnp.maximum(m, _ld32(act, run, r, RC))
                if t1 == j[1] + 1:
                    row_max[(j, r)] = jnp.max(m, axis=1, keepdims=True)
            _st32(act, run, r, m[0:8] if t1 == j[1] + 1 else m)

        st.step(lambda r: [_ld16(act, heads[n], j * T + r, RC) for (n, j), _, _ in groups[g]],
                lambda qs: [_dot_nt(q, _ld16(kv, heads[n], t0 * T, (t1 - t0) * T))
                            for q, ((n, _), t0, t1) in zip(qs, groups[g])], sink, early=1, first=False)

    def exp_job(st, g, r, slot):
        def start():
            out = []
            for j, t0, t1 in groups[g]:
                ps = [jnp.exp2(_ld32(act, A_S, s_row(j, t, r), RC) - row_max[(j, r)]) for t in range(t0, t1)]
                out.append(jnp.concatenate(ps, axis=1))
                l = _tree(jnp.add, ps)
                if t0 > 0:
                    l = l + _ld32(act, run, T + r, RC)
                if t1 == j[1] + 1:
                    inv_sum[(j, r)] = pltpu.reciprocal(jnp.sum(l, axis=1, keepdims=True), full_range=False)
            probs[(g, r)] = out
            st.at(slot + 1, lambda: _st32(act, run, T + r, l[RC - 8:] if t1 == j[1] + 1 else l))

        st.at(slot, start)

    def pv_step(st, g):
        def sink(r, res):
            for (j, t0, t1), o in zip(groups[g], res):
                if t0 > 0:
                    o = o + _ld32(act, run, 2 * T + r, RC)
                if t1 == j[1] + 1:
                    _st16(act, heads[j[0]], j[1] * T + r, o * inv_sum.pop((j, r)))
                else:
                    _st32(act, run, 2 * T + r, o)

        st.step(lambda r: probs.pop((g, r)),
                lambda ps: [_dot(p.astype(BF16), _ld16(kv, v_page[n], t0 * T, (t1 - t0) * T))
                            for p, ((n, _), t0, t1) in zip(ps, groups[g])], sink)

    need = [index[(runs[-1][0], runs[-1][0][1])] // 4 for runs in groups]
    seq, qk_pos = [], {}
    gq = gp = 0
    while gp < ng:
        ready = need[gp] in qk_pos and NC * (qk_pos[need[gp]] + DELAY) + XLAG <= NC * len(seq)
        if gq == ng or (ready and seq[-1][0] is qk_step):
            assert qk_pos[need[gp]] + DELAY <= len(seq)
            seq.append((pv_step, gp))
            gp += 1
        else:
            qk_pos[gq] = len(seq)
            seq.append((qk_step, gq))
            gq += 1
        assert (gq - gp) * 4 <= RING

    st = _Stream()
    for pos, (step, g) in enumerate(seq):
        if step is pv_step:
            for c in range(NC):
                exp_job(st, g, c * RC, NC * pos + c)
    for step, g in seq:
        step(st, g)
    st.drain()


def _kernel(x_hbm, ckv_hbm, wq_hbm, wuk_hbm, wuv_hbm, wo_hbm, bk_hbm, bv_hbm, sk_hbm,
            shift_hbm, ssmd_hbm, gate_hbm, out_hbm,
            act, kv, io_v, ckv_v, wq_v, wuk_v, wuv_v, wo_v, bk_v, bv_v, sk_v, shift_v, ssmd_v, gate_v,
            dft_v, idft_v, kpad_v, par_v, run_s, sems):
    def start(copies):
        for c in copies:
            c.start()

    def wait(copies):
        for c in copies:
            c.wait()

    def c_cp():
        return [pltpu.make_async_copy(ckv_hbm, ckv_v, sems.at[SEM_C])]

    def wkv_cp(g):
        return [pltpu.make_async_copy(src.at[:, pl.ds(g * HG, HG), :], dst.at[g], sems.at[SEM_KV])
                for src, dst in ((wuk_hbm, wuk_v), (wuv_hbm, wuv_v))]

    def a_cp():
        pairs = [(wq_hbm.at[:, pl.ds(g * HG, HG), :], wq_v.at[g]) for g in range(NG)]
        pairs += [(x_hbm.at[:, pl.ds(i * T, T)], io_v.at[i]) for i in range(NCB)] + [(gate_hbm, gate_v)]
        return [pltpu.make_async_copy(src, dst, sems.at[SEM_A]) for src, dst in pairs]

    def b_cp():
        pairs = [(shift_hbm, shift_v), (ssmd_hbm, ssmd_v)]
        for i in range(NCB):
            blk = pl.ds(i * T, T)
            pairs += [(bk_hbm.at[:, blk], bk_v.at[i]), (bv_hbm.at[:, blk], bv_v.at[i]),
                      (sk_hbm.at[blk, :], sk_v.at[i]), (wo_hbm.at[:, blk], wo_v.at[i])]
        return [pltpu.make_async_copy(src, dst, sems.at[SEM_B]) for src, dst in pairs]

    def out_cp(i):
        return [pltpu.make_async_copy(io_v.at[i], out_hbm.at[:, pl.ds(pl.multiple_of(i * T, T), T)],
                                      sems.at[SEM_O])]

    start(wkv_cp(0))

    def phase(f, n):
        return (((2 * f + 1) * n) & (4 * C - 1)).astype(F32) * (math.pi / (2 * C))

    row = lax.broadcasted_iota(jnp.int32, (C, C), 0)
    col = lax.broadcasted_iota(jnp.int32, (C, C), 1)
    dft_v[0:C, :] = jnp.cos(phase(row, col)).astype(BF16)
    dft_v[C:2 * C, :] = (-jnp.sin(phase(row, col))).astype(BF16)
    idft_v[:, 0:C] = (jnp.cos(phase(col, row)) * (1.0 / C)).astype(BF16)
    idft_v[:, C:2 * C] = (-jnp.sin(phase(col, row)) * (1.0 / C)).astype(BF16)
    kpad_v[0:8, :] = jnp.zeros((8, T), F32)
    run_s[0] = A_RUN
    start(c_cp())

    def repack_kv(g, r0, n):
        jobs = []
        for raw, row0 in ((wuk_v, M), (wuv_v, M + DC)):
            for r in range(0, n, RR):
                jobs += _repack_jobs(raw, act, g, r0 + r, row0, len(jobs) // 2)
        return jobs

    def repack_first(i, carry):
        jobs = repack_kv(0, i * 4 * RR, 4 * RR)
        for job in jobs[::2]:
            job()
        for k in range(1, len(jobs), 4):
            for fin in [job() for job in jobs[k:k + 4:2]]:
                fin()
        return carry

    def page_c(i, carry):
        rows = ckv_v[pl.ds(pl.multiple_of(i * 2 * T, 2 * T), 2 * T), :]
        for k in range(DC // T):
            act[A_C + k, pl.ds(pl.multiple_of(i * T, T), T), :] = pltpu.bitcast(rows[:, k * T:(k + 1) * T], F32)
        return carry

    def latent_project(h0, queues, nstep):
        run = run_s[0]
        st = _Stream(queues)
        nt = S // T
        for q in queues:
            q.spread((nstep * nt - 2 - DELAY) * NC - q.lag)
        pages = [h0 + (p // 2 + p % 2 * H) for p in range(2 * HP)]

        def weight(p):
            return _ld16(act, A_W + h0 + p // 2, M + p % 2 * DC, DC)

        w = {0: weight(0)}
        for n in range(nstep * nt):
            def sink(r, res, n=n):
                if n < nstep * nt - 1 - DELAY:
                    _st32(act, run, 0, res[0][0:8])
                _st16(kv, pages[n // nt], n % nt * T + r, res[0])

            if n % nt == nt - 1:
                w[n // nt + 1] = weight(n // nt + 1)
            st.step(lambda r: [jnp.concatenate([_ld16(act, A_C + k, n % nt * T + r, RC) for k in range(4)], axis=1)],
                    lambda lhs: [_dot(lhs[0], w[n // nt])], sink)
        st.drain()
        for p in range(nstep, 2 * HP):
            c = jnp.concatenate([_ld16(act, A_C + k, 0, S) for k in range(4)], axis=1)
            _st16(kv, pages[p], 0, _dot(c, w[p] if p in w else weight(p)))

    def latent_a(i, carry):
        for g in range(1, NG):
            @pl.when(i == g)
            def _():
                wait(wkv_cp(g))
                if g + 1 < NG:
                    start(wkv_cp(g + 1))
                if g == 1:
                    start(a_cp())

        jobs = _Jobs(1)
        for job in repack_kv(i, 0, DC):
            jobs.add(1, job)
        latent_project(i * HP, [jobs], 2)
        return carry

    def latent_b(i, carry):
        gate_w = gate_v[...].astype(F32)

        def page_x(r):
            rows = pl.ds(pl.multiple_of((i * (S // NG) + r) // 2, RC // 2), RC // 2)
            for cb in range(NCB):
                act[A_X + cb, rows, :] = pltpu.bitcast(
                    io_v[cb, pl.ds(pl.multiple_of(i * (S // NG) + r, RC), RC), :], F32)

        def gate(r):
            rows = pl.ds(pl.multiple_of((i * (S // NG) + r) // 2, 8), 8)
            acc = _tree(jnp.add, [pltpu.bitcast(act[A_X + cb, rows, :], BF16).astype(F32) * gate_w[cb:cb + 1, :]
                                  for cb in range(NCB)])
            g = jax.nn.sigmoid(jnp.sum(acc, axis=1, keepdims=True))

            def fin():
                act[A_GATE + i // 2, pl.ds(pl.multiple_of(i % 2 * (S // NG) + r, 16), 16), :] = (
                    jnp.broadcast_to(g, (16, T)))
            return fin

        jobs, gates = _Jobs(1), _Jobs(6)
        for k in range(M // RR):
            for job in _repack_jobs(wq_v, act, i, k * RR, 0, k):
                jobs.add(1, job)
        for r in range(0, S // NG, RC):
            for job in (lambda r=r: page_x(r), lambda r=r: gate(r), lambda r=r: gate(r + 16)):
                gates.add(1, job)
        latent_project(H // 2 + i * HP, [gates, jobs], 3)
        return carry

    def query_project(i, carry):
        scale = (D ** -0.5) * math.log2(math.e)
        w = jnp.concatenate([_ld16(act, A_W + i * HP + h, 0, M) for h in range(HP)], axis=1)
        for r0 in range(0, S, 2 * T):
            q = _dot(jnp.concatenate([io_v[cb, r0:r0 + 2 * T, :] for cb in range(NCB)], axis=1), w) * scale
            for h in range(HP):
                _st16(act, A_Q + i * HP + h, r0, q[:, h * D:(h + 1) * D])
        return carry

    wait(wkv_cp(0))
    lax.fori_loop(0, DC // (4 * RR), repack_first, 0)
    wait(c_cp())
    start(wkv_cp(1))
    lax.fori_loop(0, S // (2 * T), page_c, 0)
    lax.fori_loop(0, NG, latent_a, 0)
    wait(a_cp())
    start(b_cp())
    lax.fori_loop(0, NG, latent_b, 0)
    lax.fori_loop(0, H // HP, query_project, 0)

    def heads(i, carry):
        _attention(kv, act, run_s[0], [A_Q + i * HA + n for n in range(HA)])
        return carry

    lax.fori_loop(0, H // HA, heads, 0)
    wait(b_cp())
    shift = shift_v[...].astype(F32)
    ssmd = ssmd_v[...].astype(F32)
    for cb in range(NCB):
        par_v[cb, 0:KS, :] = shift[:, cb * T:(cb + 1) * T]
        par_v[cb, KS:KS + 1, :] = ssmd[cb:cb + 1, :]

    def spec_row(page, a, im):
        return a * 4 * C + im * (C + 8) + (page == A_G) * 16

    def out_block(cb, carry):
        run = run_s[0]
        kpad_v[8:8 + S, :] = bk_v[cb].astype(F32)
        sgn = (1 - 2 * (lax.broadcasted_iota(jnp.int32, (C, T), 0) & 1)).astype(F32)
        prev = None
        for d0 in range(0, P, 4):
            taps = jnp.concatenate([sk_v[cb, :, d * C:(d + 1) * C] for d in range(d0, d0 + 4)], axis=0)
            hf = _dot_nt(dft_v[...], taps)
            for k in range(4):
                cur = hf[0:C, k * T:(k + 1) * T], hf[C:2 * C, k * T:(k + 1) * T]
                if prev is None:
                    re, im = cur[0] + par_v[cb, KS:KS + 1, :], cur[1]
                else:
                    re, im = cur[0] - sgn * prev[1], cur[1] + sgn * prev[0]
                prev = cur
                _st32(act, A_G, spec_row(A_G, d0 + k, 0), re)
                _st32(act, A_G, spec_row(A_G, d0 + k, 1), im)
            kvs = []
            for a in range(d0, d0 + 4):
                acc = None
                for j in range(KS):
                    t = kpad_v[pl.ds(8 + a * C - j, C), :] * par_v[cb, j:j + 1, :]
                    acc = t if acc is None else acc + t
                kvs.append((acc * bv_v[cb, a * C:(a + 1) * C, :].astype(F32)).astype(BF16))
            uf = _dot(dft_v[...], jnp.concatenate(kvs, axis=1))
            for k in range(4):
                for im in range(2):
                    _st32(act, A_U, spec_row(A_U, d0 + k, im), uf[im * C:(im + 1) * C, k * T:(k + 1) * T])

        done, part = [], {}

        def spec(page, a, f0, n=MF):
            return [_ld32(act, page, spec_row(page, a, im) + f0, n) for im in range(2)]

        def mac(a, f0, b0, b1):
            acc, kept = part.pop((a, f0), ({}, {}))
            gs = {d: kept.get(d) or spec(A_G, d, f0) for d in range(max(a - b1, 0), a - b0 + 1)}
            for b in range(b0, b1):
                ur, ui = spec(A_U, b, f0)
                for o in (a, a - 1):
                    if b <= o:
                        gr, gi = gs[o - b]
                        t = ur * gr - ui * gi, ur * gi + ui * gr
                        acc[o] = (acc[o][0] + t[0], acc[o][1] + t[1]) if o in acc else t
            if b1 <= a:
                part[(a, f0)] = acc, gs
            vals = dict(acc)

            def fin():
                for o, (yr, yi) in vals.items():
                    _st32(act, A_Y, spec_row(A_Y, o, 0) + f0, yr)
                    _st32(act, A_Y, spec_row(A_Y, o, 1) + f0, yi)
                if f0 == C - MF and b1 > a:
                    done.append((a, a - 1))
            return fin

        macs, mixes = _Jobs(1), _Jobs(1)
        for a in range(P - 1, 0, -2):
            for f0 in range(0, C, MF):
                for b0 in range(0, a + 1, MB):
                    b1 = min(b0 + MB, a + 1)
                    macs.add(b1 - b0, lambda arg=(a, f0, b0, b1): mac(*arg))
        macs.spread(((P - 1) * (H // 4) - DELAY) * NC - 3)
        mixes.rate = 1.0
        st = _Stream([macs, mixes])
        attn, conv = {}, {}

        def mix(r0, a, y):
            x = _ld16(act, A_X + cb, r0, RC).astype(F32)
            g = _ld32(act, A_GATE, r0, RC)
            return lambda: _st16(act, A_STG, r0, g * a + (1.0 - g) * (x * y))

        def queue_mix(r0):
            if r0 in attn and r0 in conv:
                if not mixes.jobs:
                    mixes.credit = 0.0
                mixes.add(3, lambda arg=(r0, attn.pop(r0), conv.pop(r0)): mix(*arg))

        def out_step(a, k):
            def sink(r, res):
                acc = res[0] if k == 0 else res[0] + _ld32(act, run, r, RC)
                _st32(act, run, r, acc)
                if k == H // 4 - 1:
                    attn[a * C + r] = acc
                    queue_mix(a * C + r)

            st.step(lambda r: [jnp.concatenate([_ld16(act, A_Q + 4 * k + i, a * C + r, RC) for i in range(4)],
                                               axis=1)],
                    lambda lhs: [_dot(lhs[0], wo_v[cb, k * 4 * D:(k + 1) * 4 * D, :])], sink, early=2)

        def idft_step(pair, ys):
            def sink(r, res):
                _st32(act, run, 3 * T, res[0][0:8, 0:T])
                for i, a in enumerate(pair):
                    conv[a * C + r] = res[0][:, i * T:(i + 1) * T]
                    queue_mix(a * C + r)

            st.step(lambda r: [idft_v[r:r + RC, :]], lambda lhs: [_dot(lhs[0], ys)], sink, early=2)

        for a in reversed(range(P)):
            for k in range(H // 4):
                pair = done.pop(0) if done else None
                if pair:
                    ys = jnp.concatenate([jnp.concatenate(spec(A_Y, o, 0, C), axis=0) for o in pair],
                                         axis=1).astype(BF16)
                out_step(a, k)
                if pair:
                    idft_step(pair, ys)
        assert macs.idle() and not done
        st.drain()
        assert not attn and not conv
        io_v[cb] = _ld16(act, A_STG, 0, S)
        start(out_cp(cb))
        return carry

    lax.fori_loop(0, NCB, out_block, 0)
    for i in range(NCB):
        wait(out_cp(i))


@jax.jit
def pallas_gated_mix__compressed_kv_cla__ssm_conv_h3__prompt_kernel(
    A_x: jax.Array,
    A_c_kv: jax.Array,
    A_w_q: jax.Array,
    A_w_uk: jax.Array,
    A_w_uv: jax.Array,
    A_w_o: jax.Array,
    B_q: jax.Array,
    B_k: jax.Array,
    B_v: jax.Array,
    B_shift_k: jax.Array,
    B_ssm_k: jax.Array,
    B_ssm_D: jax.Array,
    gate_w: jax.Array,
):
    del B_q
    hbm = pl.BlockSpec(memory_space=pl.ANY)
    scratch = [
        pltpu.VMEM((A_END, PAGE, T), F32), pltpu.VMEM((2 * H, PAGE, D), F32),
        pltpu.VMEM((NCB, S, T), BF16), pltpu.VMEM((S, DC), BF16),
        pltpu.VMEM((NG, M, HG, D), BF16), pltpu.VMEM((NG, DC, HG, D), BF16), pltpu.VMEM((NG, DC, HG, D), BF16),
        pltpu.VMEM((NCB, H * D, T), BF16),
        pltpu.VMEM((NCB, S, T), BF16), pltpu.VMEM((NCB, S, T), BF16), pltpu.VMEM((NCB, T, S), BF16),
        pltpu.VMEM((KS, M), BF16), pltpu.VMEM((NCB, T), BF16), pltpu.VMEM((NCB, T), BF16),
        pltpu.VMEM((2 * C, C), BF16), pltpu.VMEM((C, 2 * C), BF16), pltpu.VMEM((S + 8, T), F32),
        pltpu.VMEM((NCB, 8, T), F32),
        pltpu.SMEM((1,), jnp.int32),
        pltpu.SemaphoreType.DMA((SEM_END,)),
    ]
    out = pl.pallas_call(
        _kernel,
        out_shape=jax.ShapeDtypeStruct((S, M), BF16),
        in_specs=[hbm] * 12,
        out_specs=hbm,
        scratch_shapes=scratch,
        compiler_params=pltpu.CompilerParams(vmem_limit_bytes=124 * 1024 * 1024),
    )(A_x.reshape(S, M), A_c_kv.reshape(S, DC), A_w_q, A_w_uk, A_w_uv, A_w_o.reshape(H * D, M),
      B_k.reshape(S, M), B_v.reshape(S, M), B_ssm_k,
      B_shift_k.T, B_ssm_D.reshape(NCB, T), gate_w.reshape(NCB, T))
    return out.reshape(1, S, M)
```

```python
import math

import jax
import jax.numpy as jnp
import numpy as np
from jax import lax
from jax.experimental import pallas as pl
from jax.experimental.pallas import tpu as pltpu

S = 2048
M = 1024
H = 32
D = 128
DC = 512
KS = 4
T = 128
C = 128
P = S // C
NCB = M // T
HG = 8
NG = H // HG

RC = 32
NC = T // RC
DELAY = 2
XLAG = 3
HP = 4
HA = 2
RR = 32
MB = 2
MF = 8
RING = 64

PAGE = S // 2
A_Q = 0
A_X = A_Q + H
A_C = A_X + NCB
A_GATE = A_C + DC // T
A_RUN = A_GATE + 2
A_STG = A_RUN + 1
A_W = A_STG + 2
A_S = A_W
A_U, A_G, A_Y = A_W, A_W + 8, A_W + 16
A_END = A_W + H
SEM_C0, SEM_C1, SEM_KV, SEM_A, SEM_B, SEM_O, SEM_END = range(7)

F32 = jnp.float32
BF16 = jnp.bfloat16
U32 = jnp.uint32


def _dot(a, b):
    return jnp.dot(a, b, preferred_element_type=F32)


def _dot_nt(a, b):
    return lax.dot_general(a, b, (((1,), (1,)), ((), ())), preferred_element_type=F32)


def _ld16(ref, page, r0, n):
    return pltpu.bitcast(ref[page, r0 // 2:(r0 + n) // 2, :], BF16)


def _st16(ref, page, r0, val):
    ref[page, r0 // 2:(r0 + val.shape[0]) // 2, :] = pltpu.bitcast(val.astype(BF16), F32)


def _ld32(ref, page, r0, n):
    return ref[page + r0 // PAGE if r0 >= PAGE else page, r0 % PAGE:r0 % PAGE + n, :]


def _st32(ref, page, r0, val):
    ref[page + r0 // PAGE if r0 >= PAGE else page, r0 % PAGE:r0 % PAGE + val.shape[0], :] = val


def _tree(op, vals):
    while len(vals) > 1:
        vals = [op(a, b) for a, b in zip(vals[::2], vals[1::2])] + vals[len(vals) // 2 * 2:]
    return vals[0]


class _Jobs:
    def __init__(self, lag):
        self.jobs, self.live = [], []
        self.lag, self.now, self.credit, self.rate = lag, 0, 0.0, 0.0

    def add(self, cost, fn):
        self.jobs.append((cost, fn))

    def spread(self, slots):
        self.rate = sum(c for c, _ in self.jobs) / slots

    def idle(self):
        return not self.jobs and not self.live

    def tick(self):
        self.now += 1
        while self.live and self.live[0][0] <= self.now:
            self.live.pop(0)[1]()
        self.credit += self.rate
        while self.jobs and self.jobs[0][0] <= self.credit + 1e-6:
            cost, fn = self.jobs.pop(0)
            self.credit -= cost
            fin = fn()
            if fin is not None:
                self.live.append((self.now + self.lag, fin))

    def flush(self):
        while self.jobs:
            fin = self.jobs.pop(0)[1]()
            if fin is not None:
                self.live.append((0, fin))
        while self.live:
            self.live.pop(0)[1]()


class _Stream:
    def __init__(self, queues=()):
        self.pos = 0
        self.events = {}
        self.queues = queues

    def at(self, slot, fn, first=False):
        assert slot >= NC * self.pos
        lst = self.events.setdefault(slot, [])
        lst.insert(0 if first else len(lst), fn)

    def step(self, load, mm, sink, early=0, first=True):
        chunks = []
        for c in range(NC):
            for fn in self.events.pop(NC * self.pos + c, ()):
                fn()
            if self.pos >= DELAY:
                for q in self.queues:
                    q.tick()
            chunks.append(load(c * RC))
        res = mm([jnp.concatenate(col, axis=0) for col in zip(*chunks)])
        for c in range(NC):
            self.at(NC * (self.pos + DELAY) + c - early, lambda r=c * RC: sink(r, [v[r:r + RC] for v in res]), first)
        self.pos += 1

    def drain(self):
        for slot in sorted(self.events):
            for fn in self.events.pop(slot):
                fn()
        for q in self.queues:
            q.flush()


def _repack_jobs(raw, act, g, r, row0, k):
    page, base = A_STG + k % 8 // 4, k % 4 * (RR * HG // 2)

    def stage():
        blk = raw[g, pl.ds(pl.multiple_of(r, RR), RR)]
        act[page, base:base + RR * HG // 2, :] = pltpu.bitcast(blk.reshape(RR * HG, D), F32)

    def split():
        out = pl.ds(pl.multiple_of((row0 + r) // 2, RR // 2), RR // 2)
        vals = []
        for hp in range(HG // 2):
            ev, od = (pltpu.bitcast(act[page, pl.ds(base + o + hp, RR // 2, stride=HG), :], U32)
                      for o in (0, HG // 2))
            vals += [(ev & np.uint32(0xFFFF)) | (od << 16), (ev >> 16) | (od & np.uint32(0xFFFF0000))]

        def fin():
            for i, v in enumerate(vals):
                act[A_W + g * HG + i, out, :] = pltpu.bitcast(v, F32)
        return fin

    return [stage, split]


def _attention(kv, act, run, heads):
    tri = lax.broadcasted_iota(jnp.int32, (T, T), 1) <= lax.broadcasted_iota(jnp.int32, (T, T), 0)
    nt = S // T
    order = [nt // 2 - 1] + [j for a in reversed(range(nt // 2 - 1)) for j in (a, nt - 2 - a)] + [nt - 1]
    tiles = [((n, j), t) for n in range(len(heads)) for j in order for t in range(j + 1)]
    index = {jt: i for i, jt in enumerate(tiles)}
    groups = []
    for g in range(len(tiles) // 4):
        runs = []
        for j, t in tiles[4 * g:4 * g + 4]:
            if runs and runs[-1][0] == j:
                runs[-1][2] += 1
            else:
                runs.append([j, t, t + 1])
        groups.append(runs)
    ng = len(groups)
    v_page = [H + h for h in heads]
    row_max, inv_sum, probs = {}, {}, {}

    def s_row(j, t, r):
        return index[(j, t)] % RING * T + r

    def qk_step(st, g):
        def sink(r, res):
            for (j, t0, t1), s in zip(groups[g], res):
                vs = []
                for t in range(t0, t1):
                    v = s[:, (t - t0) * T:(t - t0 + 1) * T]
                    if t == j[1]:
                        v = jnp.where(tri[r:r + RC], v, -jnp.inf)
                    _st32(act, A_S, s_row(j, t, r), v)
                    vs.append(v)
                m = _tree(jnp.maximum, vs)
                if t0 > 0:
                    m = jnp.maximum(m, _ld32(act, run, r, RC))
                if t1 == j[1] + 1:
                    row_max[(j, r)] = jnp.max(m, axis=1, keepdims=True)
            _st32(act, run, r, m[0:8] if t1 == j[1] + 1 else m)

        st.step(lambda r: [_ld16(act, heads[n], j * T + r, RC) for (n, j), _, _ in groups[g]],
                lambda qs: [_dot_nt(q, _ld16(kv, heads[n], t0 * T, (t1 - t0) * T))
                            for q, ((n, _), t0, t1) in zip(qs, groups[g])], sink, early=1, first=False)

    def exp_job(st, g, r, slot):
        def start():
            out = []
            for j, t0, t1 in groups[g]:
                ps = [jnp.exp2(_ld32(act, A_S, s_row(j, t, r), RC) - row_max[(j, r)]) for t in range(t0, t1)]
                out.append(jnp.concatenate(ps, axis=1))
                l = _tree(jnp.add, ps)
                if t0 > 0:
                    l = l + _ld32(act, run, T + r, RC)
                if t1 == j[1] + 1:
                    inv_sum[(j, r)] = pltpu.reciprocal(jnp.sum(l, axis=1, keepdims=True), full_range=False)
            probs[(g, r)] = out
            st.at(slot + 1, lambda: _st32(act, run, T + r, l[RC - 8:] if t1 == j[1] + 1 else l))

        st.at(slot, start)

    def pv_step(st, g):
        def sink(r, res):
            for (j, t0, t1), o in zip(groups[g], res):
                if t0 > 0:
                    o = o + _ld32(act, run, 2 * T + r, RC)
                if t1 == j[1] + 1:
                    _st16(act, heads[j[0]], j[1] * T + r, o * inv_sum.pop((j, r)))
                else:
                    _st32(act, run, 2 * T + r, o)

        st.step(lambda r: probs.pop((g, r)),
                lambda ps: [_dot(p.astype(BF16), _ld16(kv, v_page[n], t0 * T, (t1 - t0) * T))
                            for p, ((n, _), t0, t1) in zip(ps, groups[g])], sink)

    need = [index[(runs[-1][0], runs[-1][0][1])] // 4 for runs in groups]
    seq, qk_pos = [], {}
    gq = gp = 0
    while gp < ng:
        ready = need[gp] in qk_pos and NC * (qk_pos[need[gp]] + DELAY) + XLAG <= NC * len(seq)
        if gq == ng or (ready and seq[-1][0] is qk_step):
            assert qk_pos[need[gp]] + DELAY <= len(seq)
            seq.append((pv_step, gp))
            gp += 1
        else:
            qk_pos[gq] = len(seq)
            seq.append((qk_step, gq))
            gq += 1
        assert (gq - gp) * 4 <= RING

    st = _Stream()
    for pos, (step, g) in enumerate(seq):
        if step is pv_step:
            for c in range(NC):
                exp_job(st, g, c * RC, NC * pos + c)
    for step, g in seq:
        step(st, g)
    st.drain()


def _kernel(x_hbm, ckv_hbm, wq_hbm, wuk_hbm, wuv_hbm, wo_hbm, bk_hbm, bv_hbm, sk_hbm,
            shift_hbm, ssmd_hbm, gate_hbm, out_hbm,
            act, kv, io_v, ckv_v, wq_v, wuk_v, wuv_v, wo_v, bk_v, bv_v, sk_v, shift_v, ssmd_v, gate_v,
            dft_v, idft_v, kpad_v, par_v, run_s, sems):
    def start(copies):
        for c in copies:
            c.start()

    def wait(copies):
        for c in copies:
            c.wait()

    def c_cp(half):
        rows = pl.ds(half * (S // 2), S // 2)
        return [pltpu.make_async_copy(ckv_hbm.at[rows], ckv_v.at[rows], sems.at[SEM_C0 + half])]

    def wkv_cp(g):
        return [pltpu.make_async_copy(src.at[:, pl.ds(g * HG, HG), :], dst.at[g], sems.at[SEM_KV])
                for src, dst in ((wuk_hbm, wuk_v), (wuv_hbm, wuv_v))]

    def a_cp():
        pairs = [(wq_hbm.at[:, pl.ds(g * HG, HG), :], wq_v.at[g]) for g in range(NG)]
        pairs += [(x_hbm.at[:, pl.ds(i * T, T)], io_v.at[i]) for i in range(NCB)] + [(gate_hbm, gate_v)]
        return [pltpu.make_async_copy(src, dst, sems.at[SEM_A]) for src, dst in pairs]

    def b_cp():
        pairs = [(shift_hbm, shift_v), (ssmd_hbm, ssmd_v)]
        for i in range(NCB):
            blk = pl.ds(i * T, T)
            pairs += [(bk_hbm.at[:, blk], bk_v.at[i]), (bv_hbm.at[:, blk], bv_v.at[i]),
                      (sk_hbm.at[blk, :], sk_v.at[i]), (wo_hbm.at[:, blk], wo_v.at[i])]
        return [pltpu.make_async_copy(src, dst, sems.at[SEM_B]) for src, dst in pairs]

    def out_cp(i):
        return [pltpu.make_async_copy(io_v.at[i], out_hbm.at[:, pl.ds(pl.multiple_of(i * T, T), T)],
                                      sems.at[SEM_O])]

    start(wkv_cp(0))

    def phase(f, n):
        return (((2 * f + 1) * n) & (4 * C - 1)).astype(F32) * (math.pi / (2 * C))

    row = lax.broadcasted_iota(jnp.int32, (C, C), 0)
    col = lax.broadcasted_iota(jnp.int32, (C, C), 1)
    dft_v[0:C, :] = jnp.cos(phase(row, col)).astype(BF16)
    dft_v[C:2 * C, :] = (-jnp.sin(phase(row, col))).astype(BF16)
    idft_v[:, 0:C] = (jnp.cos(phase(col, row)) * (1.0 / C)).astype(BF16)
    idft_v[:, C:2 * C] = (-jnp.sin(phase(col, row)) * (1.0 / C)).astype(BF16)
    kpad_v[0:8, :] = jnp.zeros((8, T), F32)
    run_s[0] = A_RUN
    start(c_cp(0))

    def repack_kv(g, r0, n):
        jobs = []
        for raw, row0 in ((wuk_v, M), (wuv_v, M + DC)):
            for r in range(0, n, RR):
                jobs += _repack_jobs(raw, act, g, r0 + r, row0, len(jobs) // 2)
        return jobs

    def repack_first(i, carry):
        jobs = repack_kv(0, i * 4 * RR, 4 * RR)
        for job in jobs[::2]:
            job()
        for k in range(1, len(jobs), 4):
            for fin in [job() for job in jobs[k:k + 4:2]]:
                fin()
        return carry

    def page_c(half):
        def body(i, carry):
            rows = ckv_v[pl.ds(pl.multiple_of(half * (S // 2) + i * 2 * T, 2 * T), 2 * T), :]
            for k in range(DC // T):
                act[A_C + 2 * half + k // 2, pl.ds(pl.multiple_of(k % 2 * (PAGE // 2) + i * T, T), T), :] = (
                    pltpu.bitcast(rows[:, k * T:(k + 1) * T], F32))
            return carry

        lax.fori_loop(0, S // (4 * T), body, 0)

    def latent_project(i, queues, nstep):
        run = run_s[0]
        st = _Stream(queues)
        nt = S // 2 // T
        for q in queues:
            q.spread((nstep * nt - 2 - DELAY) * NC - q.lag)
        h0, half = i // 2 * HG, i % 2
        c_page = [A_C + 2 * half, A_C + 2 * half + 1]
        row0 = half * (PAGE // 2)

        def latent(r, n):
            return jnp.concatenate([_ld16(act, c_page[k // 2], k % 2 * (S // 2) + r, n) for k in range(4)], axis=1)

        def weight(p):
            return _ld16(act, A_W + h0 + p // 2, M + p % 2 * DC, DC)

        def store(p, r, val):
            rows = pl.ds(pl.multiple_of(row0 + r // 2, RC // 2), val.shape[0] // 2)
            kv[h0 + (p // 2 + p % 2 * H), rows, :] = pltpu.bitcast(val.astype(BF16), F32)

        w = {0: weight(0)}
        for n in range(nstep * nt):
            def sink(r, res, n=n):
                if n < nstep * nt - 1 - DELAY:
                    _st32(act, run, 0, res[0][0:8])
                store(n // nt, n % nt * T + r, res[0])

            if n % nt == nt - 1:
                w[n // nt + 1] = weight(n // nt + 1)
            st.step(lambda r: [latent(n % nt * T + r, RC)], lambda lhs: [_dot(lhs[0], w[n // nt])], sink)
        st.drain()
        for p in range(nstep, 2 * HG):
            store(p, 0, _dot(latent(0, S // 2), w[p] if p in w else weight(p)))

    def latent_a(i, carry):
        for g in range(1, NG):
            @pl.when(i == g)
            def _():
                wait(wkv_cp(g))
                if g + 1 < NG:
                    start(wkv_cp(g + 1))
                if g == 1:
                    start(a_cp())
                    wait(c_cp(1))
                    page_c(1)

        jobs = _Jobs(1)
        for job in repack_kv(i, 0, DC):
            jobs.add(1, job)
        latent_project(i, [jobs], 4)
        return carry

    def latent_b(i, carry):
        gate_w = gate_v[...].astype(F32)

        def page_x(r):
            rows = pl.ds(pl.multiple_of((i * (S // NG) + r) // 2, RC // 2), RC // 2)
            for cb in range(NCB):
                act[A_X + cb, rows, :] = pltpu.bitcast(
                    io_v[cb, pl.ds(pl.multiple_of(i * (S // NG) + r, RC), RC), :], F32)

        def gate(r):
            rows = pl.ds(pl.multiple_of((i * (S // NG) + r) // 2, 8), 8)
            acc = _tree(jnp.add, [pltpu.bitcast(act[A_X + cb, rows, :], BF16).astype(F32) * gate_w[cb:cb + 1, :]
                                  for cb in range(NCB)])
            g = jax.nn.sigmoid(jnp.sum(acc, axis=1, keepdims=True))

            def fin():
                act[A_GATE + i // 2, pl.ds(pl.multiple_of(i % 2 * (S // NG) + r, 16), 16), :] = (
                    jnp.broadcast_to(g, (16, T)))
            return fin

        jobs, gates = _Jobs(1), _Jobs(6)
        for k in range(M // RR):
            for job in _repack_jobs(wq_v, act, i, k * RR, 0, k):
                jobs.add(1, job)
        for r in range(0, S // NG, RC):
            for job in (lambda r=r: page_x(r), lambda r=r: gate(r), lambda r=r: gate(r + 16)):
                gates.add(1, job)
        latent_project(NG + i, [gates, jobs], 6)
        return carry

    def query_project(i, carry):
        scale = (D ** -0.5) * math.log2(math.e)
        w = jnp.concatenate([_ld16(act, A_W + i * HP + h, 0, M) for h in range(HP)], axis=1)
        for r0 in range(0, S, 2 * T):
            q = _dot(jnp.concatenate([io_v[cb, r0:r0 + 2 * T, :] for cb in range(NCB)], axis=1), w) * scale
            for h in range(HP):
                _st16(act, A_Q + i * HP + h, r0, q[:, h * D:(h + 1) * D])
        return carry

    wait(wkv_cp(0))
    lax.fori_loop(0, DC // (4 * RR), repack_first, 0)
    wait(c_cp(0))
    start(c_cp(1) + wkv_cp(1))
    page_c(0)
    lax.fori_loop(0, NG, latent_a, 0)
    wait(a_cp())
    start(b_cp())
    lax.fori_loop(0, NG, latent_b, 0)
    lax.fori_loop(0, H // HP, query_project, 0)

    def heads(i, carry):
        _attention(kv, act, run_s[0], [A_Q + i * HA + n for n in range(HA)])
        return carry

    lax.fori_loop(0, H // HA, heads, 0)
    wait(b_cp())
    shift = shift_v[...].astype(F32)
    ssmd = ssmd_v[...].astype(F32)
    for cb in range(NCB):
        par_v[cb, 0:KS, :] = shift[:, cb * T:(cb + 1) * T]
        par_v[cb, KS:KS + 1, :] = ssmd[cb:cb + 1, :]

    def spec_row(page, a, im):
        return a * 4 * C + im * (C + 8) + (page == A_G) * 16

    def out_block(cb, carry):
        run = run_s[0]
        kpad_v[8:8 + S, :] = bk_v[cb].astype(F32)
        sgn = (1 - 2 * (lax.broadcasted_iota(jnp.int32, (C, T), 0) & 1)).astype(F32)
        prev = None
        for d0 in range(0, P, 4):
            taps = jnp.concatenate([sk_v[cb, :, d * C:(d + 1) * C] for d in range(d0, d0 + 4)], axis=0)
            hf = _dot_nt(dft_v[...], taps)
            for k in range(4):
                cur = hf[0:C, k * T:(k + 1) * T], hf[C:2 * C, k * T:(k + 1) * T]
                if prev is None:
                    re, im = cur[0] + par_v[cb, KS:KS + 1, :], cur[1]
                else:
                    re, im = cur[0] - sgn * prev[1], cur[1] + sgn * prev[0]
                prev = cur
                _st32(act, A_G, spec_row(A_G, d0 + k, 0), re)
                _st32(act, A_G, spec_row(A_G, d0 + k, 1), im)
            kvs = []
            for a in range(d0, d0 + 4):
                acc = None
                for j in range(KS):
                    t = kpad_v[pl.ds(8 + a * C - j, C), :] * par_v[cb, j:j + 1, :]
                    acc = t if acc is None else acc + t
                kvs.append((acc * bv_v[cb, a * C:(a + 1) * C, :].astype(F32)).astype(BF16))
            uf = _dot(dft_v[...], jnp.concatenate(kvs, axis=1))
            for k in range(4):
                for im in range(2):
                    _st32(act, A_U, spec_row(A_U, d0 + k, im), uf[im * C:(im + 1) * C, k * T:(k + 1) * T])

        done, part = [], {}

        def spec(page, a, f0, n=MF):
            return [_ld32(act, page, spec_row(page, a, im) + f0, n) for im in range(2)]

        def mac(a, f0, b0, b1):
            acc, kept = part.pop((a, f0), ({}, {}))
            gs = {d: kept.get(d) or spec(A_G, d, f0) for d in range(max(a - b1, 0), a - b0 + 1)}
            for b in range(b0, b1):
                ur, ui = spec(A_U, b, f0)
                for o in (a, a - 1):
                    if b <= o:
                        gr, gi = gs[o - b]
                        t = ur * gr - ui * gi, ur * gi + ui * gr
                        acc[o] = (acc[o][0] + t[0], acc[o][1] + t[1]) if o in acc else t
            if b1 <= a:
                part[(a, f0)] = acc, gs
            vals = dict(acc)

            def fin():
                for o, (yr, yi) in vals.items():
                    _st32(act, A_Y, spec_row(A_Y, o, 0) + f0, yr)
                    _st32(act, A_Y, spec_row(A_Y, o, 1) + f0, yi)
                if f0 == C - MF and b1 > a:
                    done.append((a, a - 1))
            return fin

        macs, mixes = _Jobs(1), _Jobs(1)
        for a in range(P - 1, 0, -2):
            for f0 in range(0, C, MF):
                for b0 in range(0, a + 1, MB):
                    b1 = min(b0 + MB, a + 1)
                    macs.add(b1 - b0, lambda arg=(a, f0, b0, b1): mac(*arg))
        macs.spread(((P - 1) * (H // 4) - DELAY) * NC - 3)
        mixes.rate = 1.0
        st = _Stream([macs, mixes])
        attn, conv, mixed = {}, {}, []

        def mix(r0, a, y):
            x = _ld16(act, A_X + cb, r0, RC).astype(F32)
            g = _ld32(act, A_GATE, r0, RC)

            def fin():
                _st16(act, A_STG, r0, g * a + (1.0 - g) * (x * y))
                mixed.append(r0)
            return fin

        def copy_mixed(n):
            for r0 in mixed[:n]:
                io_v[cb, r0:r0 + RC, :] = _ld16(act, A_STG, r0, RC)
            del mixed[:n]

        def queue_mix(r0):
            if r0 in attn and r0 in conv:
                if not mixes.jobs:
                    mixes.credit = 0.0
                mixes.add(3, lambda arg=(r0, attn.pop(r0), conv.pop(r0)): mix(*arg))

        def out_step(a, k):
            def sink(r, res):
                acc = res[0] if k == 0 else res[0] + _ld32(act, run, r, RC)
                _st32(act, run, r, acc)
                if k == H // 4 - 1:
                    attn[a * C + r] = acc
                    queue_mix(a * C + r)

            st.step(lambda r: [jnp.concatenate([_ld16(act, A_Q + 4 * k + i, a * C + r, RC) for i in range(4)],
                                               axis=1)],
                    lambda lhs: [_dot(lhs[0], wo_v[cb, k * 4 * D:(k + 1) * 4 * D, :])], sink, early=2)

        def idft_step(pair, ys):
            def sink(r, res):
                _st32(act, run, 3 * T, res[0][0:8, 0:T])
                for i, a in enumerate(pair):
                    conv[a * C + r] = res[0][:, i * T:(i + 1) * T]
                    queue_mix(a * C + r)

            st.step(lambda r: [idft_v[r:r + RC, :]], lambda lhs: [_dot(lhs[0], ys)], sink, early=2)

        for a in reversed(range(P)):
            for k in range(H // 4):
                pair = done.pop(0) if done else None
                if pair:
                    ys = jnp.concatenate([jnp.concatenate(spec(A_Y, o, 0, C), axis=0) for o in pair],
                                         axis=1).astype(BF16)
                if a == 0 and k >= H // 4 - 4:
                    copy_mixed(S // RC // 4)
                out_step(a, k)
                if pair:
                    idft_step(pair, ys)
        assert macs.idle() and not done
        st.drain()
        assert not attn and not conv
        copy_mixed(S // RC)
        start(out_cp(cb))
        return carry

    lax.fori_loop(0, NCB, out_block, 0)
    for i in range(NCB):
        wait(out_cp(i))


@jax.jit
def pallas_gated_mix__compressed_kv_cla__ssm_conv_h3__prompt_kernel(
    A_x: jax.Array,
    A_c_kv: jax.Array,
    A_w_q: jax.Array,
    A_w_uk: jax.Array,
    A_w_uv: jax.Array,
    A_w_o: jax.Array,
    B_q: jax.Array,
    B_k: jax.Array,
    B_v: jax.Array,
    B_shift_k: jax.Array,
    B_ssm_k: jax.Array,
    B_ssm_D: jax.Array,
    gate_w: jax.Array,
):
    del B_q
    hbm = pl.BlockSpec(memory_space=pl.ANY)
    scratch = [
        pltpu.VMEM((A_END, PAGE, T), F32), pltpu.VMEM((2 * H, PAGE, D), F32),
        pltpu.VMEM((NCB, S, T), BF16), pltpu.VMEM((S, DC), BF16),
        pltpu.VMEM((NG, M, HG, D), BF16), pltpu.VMEM((NG, DC, HG, D), BF16), pltpu.VMEM((NG, DC, HG, D), BF16),
        pltpu.VMEM((NCB, H * D, T), BF16),
        pltpu.VMEM((NCB, S, T), BF16), pltpu.VMEM((NCB, S, T), BF16), pltpu.VMEM((NCB, T, S), BF16),
        pltpu.VMEM((KS, M), BF16), pltpu.VMEM((NCB, T), BF16), pltpu.VMEM((NCB, T), BF16),
        pltpu.VMEM((2 * C, C), BF16), pltpu.VMEM((C, 2 * C), BF16), pltpu.VMEM((S + 8, T), F32),
        pltpu.VMEM((NCB, 8, T), F32),
        pltpu.SMEM((1,), jnp.int32),
        pltpu.SemaphoreType.DMA((SEM_END,)),
    ]
    out = pl.pallas_call(
        _kernel,
        out_shape=jax.ShapeDtypeStruct((S, M), BF16),
        in_specs=[hbm] * 12,
        out_specs=hbm,
        scratch_shapes=scratch,
        compiler_params=pltpu.CompilerParams(vmem_limit_bytes=124 * 1024 * 1024),
    )(A_x.reshape(S, M), A_c_kv.reshape(S, DC), A_w_q, A_w_uk, A_w_uv, A_w_o.reshape(H * D, M),
      B_k.reshape(S, M), B_v.reshape(S, M), B_ssm_k,
      B_shift_k.T, B_ssm_D.reshape(NCB, T), gate_w.reshape(NCB, T))
    return out.reshape(1, S, M)
```
